```python
import os as _os
_os.environ.setdefault("JAX_PLATFORMS", "cpu")
import jax
import jax.numpy as jnp

def _softmax(x, axis=-1):
    return jax.nn.softmax(x, axis=axis)
def _gelu(x):
    return jax.nn.gelu(x, approximate=True)
def _silu(x):
    return jax.nn.silu(x)
def _sigmoid(x):
    return jax.nn.sigmoid(x)
def _layernorm(x, axis=-1, eps=1e-5):
    m = jnp.mean(x, axis=axis, keepdims=True)
    v = jnp.var(x, axis=axis, keepdims=True)
    return (x - m) / jnp.sqrt(v + eps)
def _scatter_add(tgt, idx, src, axis=0):
    return tgt.at[idx].add(src)
def _segment_sum(src, seg, n):
    return jax.ops.segment_sum(src, seg, n)
class _Rng:
    def __init__(self, key):
        self._k = key
    def _next(self):
        self._k, sub = jax.random.split(self._k)
        return sub
    def normal(self, shape):
        return jax.random.normal(self._next(), shape, dtype=jnp.bfloat16)
    def randint(self, lo, hi, shape):
        return jax.random.randint(self._next(), shape, lo, hi, dtype=jnp.int32)
    def uniform(self, shape, lo=0.0, hi=1.0):
        return jax.random.uniform(self._next(), shape, jnp.bfloat16, lo, hi)
    def permutation(self, n):
        return jax.random.permutation(self._next(), n)


kernel_name = 'sequential_preLN__mha_block__swiglu_ffn__prompt'

def setup_inputs():
    _rng = _Rng(jax.random.key(int.from_bytes(__import__("os").urandom(4), "little")))
    _w = (lambda a: (lambda t: t.astype(jnp.bfloat16) if jnp.issubdtype(t.dtype, jnp.floating) else t)(jnp.asarray(a)))
    def _A_setup():
        B, S, D, H = 1, 2048, 640, 32
        return {
            "x": _w((lambda *s: _rng.normal(s) * 0.05)(B, S, D)),
            "wqkv": _w((lambda *s: _rng.normal(s) * 0.05)(D, 3 * D)),
            "wo": _w((lambda *s: _rng.normal(s) * 0.05)(D, D)),
        }
    _A_in = _A_setup()

    def _B_setup():
        B, S, D, F = 1, 2048, 640, 1728
        return {
            "x": _w((lambda *s: _rng.normal(s) * 0.05)(B, S, D)),
            "w_gate": _w((lambda *s: _rng.normal(s) * 0.05)(D, F)),
            "w_up": _w((lambda *s: _rng.normal(s) * 0.05)(D, F)),
            "w_down": _w((lambda *s: _rng.normal(s) * 0.05)(F, D)),
        }
    _B_in = _B_setup()

    return {
        "A_x": _A_in["x"],
        "A_wqkv": _A_in["wqkv"],
        "A_wo": _A_in["wo"],
        "B_x": _B_in["x"],
        "B_w_gate": _B_in["w_gate"],
        "B_w_up": _B_in["w_up"],
        "B_w_down": _B_in["w_down"],
    }

def reference(A_x, A_wqkv, A_wo, B_x, B_w_gate, B_w_up, B_w_down):
    def _A_ref(x, wqkv, wo):
        B, S, D = x.shape
        H = 32
        Dh = D // H
        qkv = (lambda x, *d: x.transpose(*d))((x @ wqkv).reshape(B, S, 3, H, Dh), 2, 0, 3, 1, 4)
        q, k, v = qkv[0], qkv[1], qkv[2]
        scores = jnp.einsum("bhqd,bhkd->bhqk", q, k) * (Dh ** -0.5)
        p = _softmax(scores, axis=-1)
        o = jnp.einsum("bhqk,bhkd->bhqd", p, v)
        return (lambda x, *d: x.transpose(*d))(o, 0, 2, 1, 3).reshape(B, S, D) @ wo

    def _B_ref(x, w_gate, w_up, w_down):
        g = _silu(x @ w_gate)
        u = x @ w_up
        return (g * u) @ w_down

    x = A_x
    h = x + _A_ref(_layernorm(x, axis=-1), A_wqkv, A_wo)
    h2 = h + _B_ref(_layernorm(h, axis=-1), B_w_gate, B_w_up, B_w_down)
    return h2
```

```python
import math

import jax
import jax.numpy as jnp
import jax.experimental.pallas as pl
import jax.experimental.pallas.tpu as pltpu

_H = 32
_EPS = 1e-5
_RB = 512
_QB = 512
_KC = 512
_HPT = 6


def _layernorm(x):
    m = jnp.mean(x, axis=-1, keepdims=True)
    xc = x - m
    v = jnp.mean(xc * xc, axis=-1, keepdims=True)
    return xc * jax.lax.rsqrt(v + _EPS)


@jax.jit
def pallas_sequential_preLN__mha_block__swiglu_ffn__prompt_kernel(
    A_x: jax.Array,
    A_wqkv: jax.Array,
    A_wo: jax.Array,
    B_x: jax.Array,
    B_w_gate: jax.Array,
    B_w_up: jax.Array,
    B_w_down: jax.Array,
):
    del B_x
    _, S, D = A_x.shape
    F = B_w_gate.shape[1]
    Dh = D // _H
    NT = -(-_H // _HPT)
    starts = [min(_HPT * Dh * t, D - 128) for t in range(NT)]
    NQ = S // _QB
    NP = _H // 2
    NRB = S // _RB
    qscale = (Dh ** -0.5) * math.log2(math.e)
    f32, bf16 = jnp.float32, jnp.bfloat16
    NN = (((1,), (0,)), ((), ()))
    NTd = (((1,), (1,)), ((), ()))

    def kernel(x_hbm, wqkv_hbm, wo_hbm, wg_hbm, wu_hbm, wd_hbm, out_hbm,
               x_v, wqkv_v, wo_v, wg_v, wu_v, wd_v, out_v,
               wqvT, wk_w, k_s, qT_s, vT_s, oT_s, sA, sB, qA, qB,
               sem_x, sem_w, sem_o):
        def x_copy(i):
            return pltpu.make_async_copy(
                x_hbm.at[pl.ds(i * _RB, _RB)], x_v.at[pl.ds(i * _RB, _RB)], sem_x.at[i])

        w_copies = [
            pltpu.make_async_copy(wqkv_hbm, wqkv_v, sem_w.at[0]),
            pltpu.make_async_copy(wo_hbm, wo_v, sem_w.at[1]),
            pltpu.make_async_copy(wg_hbm, wg_v, sem_w.at[2]),
            pltpu.make_async_copy(wu_hbm, wu_v, sem_w.at[3]),
            pltpu.make_async_copy(wd_hbm, wd_v, sem_w.at[4]),
        ]
        w_copies[0].start()
        for i in range(NRB):
            x_copy(i).start()
        for c in w_copies[1:]:
            c.start()
        w_copies[0].wait()

        wqvT[0:D, :] = wqkv_v[:, 0:D].astype(f32).T.astype(bf16)
        wqvT[D:2 * D, :] = wqkv_v[:, 2 * D:3 * D].astype(f32).T.astype(bf16)
        wk = wqkv_v[:, D:2 * D].astype(f32)
        for t in range(NT):
            wk_w[:, t * 128:(t + 1) * 128] = wk[:, starts[t]:starts[t] + 128].astype(bf16)

        def proj(i, _):
            x_copy(i).wait()
            r0 = pl.multiple_of(i * _RB, _RB)
            xn = _layernorm(x_v[pl.ds(r0, _RB), :].astype(f32)).astype(bf16)
            kk = jax.lax.dot_general(xn, wk_w[...], NN, preferred_element_type=f32)
            for t in range(NT):
                k_s[t, pl.ds(r0, _RB), :] = kk[:, t * 128:(t + 1) * 128].astype(bf16)
            qT = jax.lax.dot_general(wqvT[0:D, :], xn, NTd, preferred_element_type=f32) * qscale
            for t in range(NT):
                qT_s[t, :, pl.ds(r0, _RB)] = qT[starts[t]:starts[t] + 128, :].astype(bf16)
            vT = jax.lax.dot_general(wqvT[D:2 * D, :], xn, NTd, preferred_element_type=f32)
            ones = jnp.ones((8, _RB), f32)
            for p in range(NP):
                for e in range(2):
                    a = 2 * Dh * p + 16 * e
                    vT_s[2 * p + e, :, pl.ds(r0, _RB)] = jnp.concatenate(
                        [vT[a:a + 24, :], ones], axis=0).astype(bf16)

        jax.lax.fori_loop(0, NRB, proj, None)

        def load_q(q_dst, h, q0):
            t = jnp.minimum(h // _HPT, NT - 1)
            off = h * Dh - jnp.minimum(t * (_HPT * Dh), D - 128)
            rows = jax.lax.broadcasted_iota(jnp.int32, (128, _QB), 0)
            qw = qT_s[t, :, pl.ds(q0, _QB)].astype(f32)
            q_dst[...] = jnp.where((rows >= off) & (rows < off + Dh), qw, 0.0).astype(bf16)
            return t

        def qk_chunk(c, t, q_src, s_dst, m):
            s = jax.lax.dot_general(k_s[t, pl.ds(c * _KC, _KC), :], q_src[...], NN,
                                    preferred_element_type=f32)
            s_dst[pl.ds(c * _KC, _KC), :] = s
            mc = jnp.max(s.reshape(_KC // 8, 8, _QB), axis=0)
            return mc if m is None else jnp.maximum(m, mc)

        def pv_chunk(c, h, s_src, m, acc):
            p = jnp.exp2(s_src[pl.ds(c * _KC, _KC), :] - m).astype(bf16)
            o = jax.lax.dot_general(vT_s[h, :, pl.ds(c * _KC, _KC)], p, NN,
                                    preferred_element_type=f32)
            return o if acc is None else acc + o

        def step(h_cur, s_cur, m_cur, h_nxt, q0_nxt, q_nxt, s_nxt):
            t = load_q(q_nxt, h_nxt, q0_nxt)
            m, acc = None, None
            for c in range(S // _KC):
                m = qk_chunk(c, t, q_nxt, s_nxt, m)
                acc = pv_chunk(c, h_cur, s_cur, m_cur, acc)
            inv = 1.0 / acc[24:32, :]
            o = [acc[8 * j:8 * j + 8, :] * inv for j in range(3)]
            return jnp.max(m, axis=0, keepdims=True), o

        t0 = load_q(qA, 0, 0)
        m0 = None
        for c in range(S // _KC):
            m0 = qk_chunk(c, t0, qA, sA, m0)
        m0 = jnp.max(m0, axis=0, keepdims=True)

        def pair(i, mA):
            p = i % NP
            q0 = pl.multiple_of((i // NP) * _QB, _QB)
            i2 = jnp.minimum(i + 1, NQ * NP - 1)
            q0n = pl.multiple_of((i2 // NP) * _QB, _QB)
            mB, oe = step(2 * p, sA, mA, 2 * p + 1, q0, qB, sB)
            mA2, oo = step(2 * p + 1, sB, mB, 2 * (i2 % NP), q0n, qA, sA)
            sub = jax.lax.broadcasted_iota(jnp.int32, (8, _QB), 0)
            mid = jnp.where(sub < Dh - 16, oe[2], oo[0])
            oT_s[pl.ds(pl.multiple_of(p * 2 * Dh, 8), 2 * Dh), pl.ds(q0, _QB)] = (
                jnp.concatenate([oe[0], oe[1], mid, oo[1], oo[2]], axis=0))
            return mA2

        jax.lax.fori_loop(0, NQ * NP, pair, m0)

        for c in w_copies[1:]:
            c.wait()

        def out_copy(i):
            return pltpu.make_async_copy(
                out_v.at[pl.ds(i * _RB, _RB)], out_hbm.at[pl.ds(i * _RB, _RB)], sem_o.at[i])

        def post(i, _):
            r0 = pl.multiple_of(i * _RB, _RB)
            o = oT_s[:, pl.ds(r0, _RB)].T.astype(bf16)
            h = x_v[pl.ds(r0, _RB), :].astype(f32) + jax.lax.dot_general(
                o, wo_v[...], NN, preferred_element_type=f32)
            hn = _layernorm(h).astype(bf16)
            g = jax.lax.dot_general(hn, wg_v[...], NTd, preferred_element_type=f32)
            u = jax.lax.dot_general(hn, wu_v[...], NTd, preferred_element_type=f32)
            a = (g * jax.nn.sigmoid(g) * u).astype(bf16)
            y = h + jax.lax.dot_general(a, wd_v[...], NN, preferred_element_type=f32)
            out_v[pl.ds(r0, _RB), :] = y.astype(bf16)
            out_copy(i).start()

        jax.lax.fori_loop(0, NRB, post, None)
        for i in range(NRB):
            out_copy(i).wait()

    anyspec = pl.BlockSpec(memory_space=pltpu.HBM)
    out = pl.pallas_call(
        kernel,
        out_shape=jax.ShapeDtypeStruct((S, D), bf16),
        in_specs=[anyspec] * 6,
        out_specs=anyspec,
        scratch_shapes=[
            pltpu.VMEM((S, D), bf16), pltpu.VMEM((D, 3 * D), bf16), pltpu.VMEM((D, D), bf16),
            pltpu.VMEM((F, D), bf16), pltpu.VMEM((F, D), bf16), pltpu.VMEM((F, D), bf16),
            pltpu.VMEM((S, D), bf16),
            pltpu.VMEM((2 * D, D), bf16), pltpu.VMEM((D, NT * 128), bf16),
            pltpu.VMEM((NT, S, 128), bf16), pltpu.VMEM((NT, 128, S), bf16),
            pltpu.VMEM((_H, 32, S), bf16), pltpu.VMEM((D, S), f32),
            pltpu.VMEM((S, _QB), f32), pltpu.VMEM((S, _QB), f32),
            pltpu.VMEM((128, _QB), bf16), pltpu.VMEM((128, _QB), bf16),
            pltpu.SemaphoreType.DMA((NRB,)), pltpu.SemaphoreType.DMA((5,)),
            pltpu.SemaphoreType.DMA((NRB,)),
        ],
        compiler_params=pltpu.CompilerParams(vmem_limit_bytes=100 * 1024 * 1024),
    )(A_x.reshape(S, D), A_wqkv, A_wo, B_w_gate.T, B_w_up.T, B_w_down)
    return out.reshape(1, S, D)
```

```python
import math

import jax
import jax.numpy as jnp
import jax.experimental.pallas as pl
import jax.experimental.pallas.tpu as pltpu

_H = 32
_EPS = 1e-5
_RB = 512
_QB = 512
_KC = 128
_SH = 2 * _KC
_HPT = 6


def _layernorm(x):
    m = jnp.mean(x, axis=-1, keepdims=True)
    xc = x - m
    v = jnp.mean(xc * xc, axis=-1, keepdims=True)
    return xc * jax.lax.rsqrt(v + _EPS)


@jax.jit
def pallas_sequential_preLN__mha_block__swiglu_ffn__prompt_kernel(
    A_x: jax.Array,
    A_wqkv: jax.Array,
    A_wo: jax.Array,
    B_x: jax.Array,
    B_w_gate: jax.Array,
    B_w_up: jax.Array,
    B_w_down: jax.Array,
):
    del B_x
    _, S, D = A_x.shape
    F = B_w_gate.shape[1]
    FM = F // 128 * 128
    FT = F - FM
    Dh = D // _H
    NT = -(-_H // _HPT)
    starts = [min(_HPT * Dh * t, D - 128) for t in range(NT)]
    NQ = S // _QB
    NP = _H // 2
    NRB = S // _RB
    qscale = (Dh ** -0.5) * math.log2(math.e)
    f32, bf16 = jnp.float32, jnp.bfloat16
    NN = (((1,), (0,)), ((), ()))
    NTd = (((1,), (1,)), ((), ()))

    def kernel(x_hbm, wqkv_hbm, wo_hbm, wg_hbm, wu_hbm, wd_hbm, out_hbm,
               x_v, wqkv_v, wo_v, wgu_v, wd_v, out_v,
               wqvT, wk_w, k_s, qT_s, vT_s, oT_s, s_s,
               sem_x, sem_w, sem_o):
        def x_copy(i):
            return pltpu.make_async_copy(
                x_hbm.at[pl.ds(i * _RB, _RB)], x_v.at[pl.ds(i * _RB, _RB)], sem_x.at[i])

        qkv_copies = [
            pltpu.make_async_copy(wqkv_hbm.at[:, pl.ds(j * D, D)], wqkv_v.at[:, pl.ds(j * D, D)],
                                  sem_w.at[j]) for j in range(3)]
        w_copies = [
            pltpu.make_async_copy(wo_hbm, wo_v, sem_w.at[3]),
            pltpu.make_async_copy(wg_hbm.at[pl.ds(0, FM)], wgu_v.at[pl.ds(0, FM)], sem_w.at[4]),
            pltpu.make_async_copy(wu_hbm.at[pl.ds(0, FM)], wgu_v.at[pl.ds(FM, FM)], sem_w.at[5]),
            pltpu.make_async_copy(wg_hbm.at[pl.ds(FM, FT)], wgu_v.at[pl.ds(2 * FM, FT)], sem_w.at[6]),
            pltpu.make_async_copy(wu_hbm.at[pl.ds(FM, FT)], wgu_v.at[pl.ds(2 * FM + FT, FT)], sem_w.at[7]),
            pltpu.make_async_copy(wd_hbm, wd_v, sem_w.at[8]),
        ]
        for j in (0, 2, 1):
            qkv_copies[j].start()
        x_copy(0).start()

        def zero_q(i, _):
            qT_s[i] = jnp.zeros((128, _QB), bf16)

        jax.lax.fori_loop(0, NQ * _H, zero_q, None)

        qkv_copies[0].wait()
        wqvT[0:D, :] = wqkv_v[:, 0:D].astype(f32).T.astype(bf16)
        qkv_copies[2].wait()
        wqvT[D:2 * D, :] = wqkv_v[:, 2 * D:3 * D].astype(f32).T.astype(bf16)
        qkv_copies[1].wait()
        for i in range(1, NRB):
            x_copy(i).start()
        for c in w_copies:
            c.start()
        wk = wqkv_v[:, D:2 * D].astype(f32)
        for t in range(NT):
            wk_w[:, t * 128:(t + 1) * 128] = wk[:, starts[t]:starts[t] + 128].astype(bf16)

        def proj(i, _):
            x_copy(i).wait()
            r0 = pl.multiple_of(i * _RB, _RB)
            xn = _layernorm(x_v[pl.ds(r0, _RB), :].astype(f32)).astype(bf16)
            kk = jax.lax.dot_general(xn, wk_w[...], NN, preferred_element_type=f32)
            for t in range(NT):
                k_s[t, pl.ds(r0, _RB), :] = kk[:, t * 128:(t + 1) * 128].astype(bf16)
            qT = jax.lax.dot_general(wqvT[0:D, :], xn, NTd, preferred_element_type=f32) * qscale
            sub = jax.lax.broadcasted_iota(jnp.int32, (8, _RB), 0)
            zero = jnp.zeros((8, _RB), f32)
            for h in range(_H):
                lo, hi = h * Dh, (h + 1) * Dh
                parts = []
                w0 = starts[h // _HPT]
                a0, a1 = (lo - w0) // 16 * 16, -(-(hi - w0) // 16) * 16
                for a in range(w0 + a0, w0 + a1, 8):
                    if a + 8 <= lo or a >= hi:
                        parts.append(zero)
                    elif a >= lo and a + 8 <= hi:
                        parts.append(qT[a:a + 8, :])
                    else:
                        parts.append(jnp.where((sub >= lo - a) & (sub < hi - a), qT[a:a + 8, :], 0.0))
                qT_s[i * _H + h, a0:a1, :] = jnp.concatenate(parts, axis=0).astype(bf16)
            vT = jax.lax.dot_general(wqvT[D:2 * D, :], xn, NTd, preferred_element_type=f32)
            for p in range(NP):
                for e in range(2):
                    a = 2 * Dh * p + 16 * e
                    v = [vT[a + 8 * j:a + 8 * j + 8, :] for j in range(3)]
                    if e == 0:
                        v[2] = jnp.where(sub < Dh - 16, v[2], 1.0)
                    else:
                        v[0] = jnp.where(sub >= 24 - Dh, v[0], 1.0)
                    vT_s[2 * p + e, :, pl.ds(r0, _RB)] = jnp.concatenate(v, axis=0)

        jax.lax.fori_loop(0, NRB, proj, None)

        def qk_chunk(c, t, q_src, s_dst, m, z=0):
            s = jax.lax.dot_general(k_s[t, pl.ds(c * _KC, _KC), :], q_src[...], NN,
                                    preferred_element_type=f32)
            s_dst[pl.ds(z + c * _KC, _KC), :] = s
            mc = jnp.max(s.reshape(_KC // 8, 8, _QB), axis=0)
            return mc if m is None else jnp.maximum(m, mc)

        def pv_chunk(c, h, s_src, m, acc, z=0):
            p = jnp.exp2(s_src[pl.ds(z + c * _KC, _KC), :] - m)
            o = jax.lax.dot_general(vT_s[h, :, pl.ds(c * _KC, _KC)], p, NN,
                                    preferred_element_type=f32)
            return o if acc is None else acc + o

        NC = S // _KC

        m0 = None
        for c in range(NC):
            m0 = qk_chunk(c, 0, qT_s.at[0], s_s, m0, _SH)

        def step(i, m_cur, even, last=False):
            m_cur = jnp.max(m_cur, axis=0, keepdims=True)
            i1 = i + 1
            t = ((i1 & (_H - 1)) * 43) >> 8
            m, acc = None, None
            for c in (range(NC) if even else reversed(range(NC))):
                if not last:
                    m = qk_chunk(c, t, qT_s.at[i1], s_s, m, 0 if even else _SH)
                acc = pv_chunk(c, i & (_H - 1), s_s, m_cur, acc, _SH if even else 0)
            oT_s[i] = acc
            return m

        def steps(j, m):
            for u in range(6):
                m = step(j * 6 + u, m, u % 2 == 0)
            return m

        n_it = (NQ * _H - 1) // 6
        m0 = jax.lax.fori_loop(0, n_it, steps, m0)
        for i in range(n_it * 6, NQ * _H):
            m0 = step(i, m0, i % 2 == 0, last=i == NQ * _H - 1)

        for c in w_copies:
            c.wait()

        def out_copy(i):
            return pltpu.make_async_copy(
                out_v.at[pl.ds(i * _RB, _RB)], out_hbm.at[pl.ds(i * _RB, _RB)], sem_o.at[i])

        def post(i, _):
            r0 = pl.multiple_of(i * _RB, _RB)
            sub = jax.lax.broadcasted_iota(jnp.int32, (8, _RB), 0)
            parts = []
            for p in range(NP):
                oe = oT_s[i * _H + 2 * p]
                oo = oT_s[i * _H + 2 * p + 1]
                oe = oe * (1.0 / oe[Dh:Dh + 1])
                oo = oo * (1.0 / oo[0:1])
                parts += [oe[0:16], jnp.where(sub < Dh - 16, oe[16:24], oo[0:8]), oo[8:24]]
            o = jnp.concatenate(parts, axis=0).T.astype(bf16)
            hs = [x_v[pl.ds(r0 + j, 128), :].astype(f32) + jax.lax.dot_general(
                o[j:j + 128], wo_v[...], NN, preferred_element_type=f32) for j in range(0, _RB, 128)]
            h = jnp.concatenate(hs, axis=0)
            hn = jnp.concatenate([_layernorm(v).astype(bf16) for v in hs], axis=0)
            gu = jax.lax.dot_general(hn, wgu_v[...], NTd, preferred_element_type=f32)
            g = jnp.concatenate([gu[:, 0:FM], gu[:, 2 * FM:2 * FM + FT]], axis=1)
            u = jnp.concatenate([gu[:, FM:2 * FM], gu[:, 2 * FM + FT:]], axis=1)
            a = (g * jax.nn.sigmoid(g) * u).astype(bf16)
            y = h + jax.lax.dot_general(a, wd_v[...], NN, preferred_element_type=f32)
            out_v[pl.ds(r0, _RB), :] = y.astype(bf16)
            out_copy(i).start()

        jax.lax.fori_loop(0, NRB, post, None)
        for i in range(NRB):
            out_copy(i).wait()

    anyspec = pl.BlockSpec(memory_space=pltpu.HBM)
    out = pl.pallas_call(
        kernel,
        out_shape=jax.ShapeDtypeStruct((S, D), bf16),
        in_specs=[anyspec] * 6,
        out_specs=anyspec,
        scratch_shapes=[
            pltpu.VMEM((S, D), bf16), pltpu.VMEM((D, 3 * D), bf16), pltpu.VMEM((D, D), bf16),
            pltpu.VMEM((2 * F, D), bf16), pltpu.VMEM((F, D), bf16),
            pltpu.VMEM((S, D), bf16),
            pltpu.VMEM((2 * D, D), bf16), pltpu.VMEM((D, NT * 128), bf16),
            pltpu.VMEM((NT, S, 128), bf16), pltpu.VMEM((NQ * _H, 128, _QB), bf16),
            pltpu.VMEM((_H, 24, S), f32), pltpu.VMEM((NQ * _H, 24, _QB), f32),
            pltpu.VMEM((S + _SH, _QB), f32),
            pltpu.SemaphoreType.DMA((NRB,)), pltpu.SemaphoreType.DMA((9,)),
            pltpu.SemaphoreType.DMA((NRB,)),
        ],
        compiler_params=pltpu.CompilerParams(vmem_limit_bytes=100 * 1024 * 1024),
    )(A_x.reshape(S, D), A_wqkv, A_wo, B_w_gate.T, B_w_up.T, B_w_down)
    return out.reshape(1, S, D)
```
